```python
import os as _os
_os.environ.setdefault('JAX_PLATFORMS', 'cpu')
import jax
import jax.numpy as jnp

def _softmax(x, axis=-1):
    return jax.nn.softmax(x, axis=axis)

def _gelu(x):
    return jax.nn.gelu(x, approximate=True)

def _silu(x):
    return jax.nn.silu(x)

def _sigmoid(x):
    return jax.nn.sigmoid(x)

def _layernorm(x, axis=-1, eps=1e-05):
    m = jnp.mean(x, axis=axis, keepdims=True)
    v = jnp.var(x, axis=axis, keepdims=True)
    return (x - m) / jnp.sqrt(v + eps)

def _scatter_add(tgt, idx, src, axis=0):
    return tgt.at[idx].add(src)

def _segment_sum(src, seg, n):
    return jax.ops.segment_sum(src, seg, n)

class _Rng:

    def __init__(self, key):
        self._k = key

    def _next(self):
        self._k, sub = jax.random.split(self._k)
        return sub

    def normal(self, shape):
        return jax.random.normal(self._next(), shape, dtype=jnp.bfloat16)

    def randint(self, lo, hi, shape):
        return jax.random.randint(self._next(), shape, lo, hi, dtype=jnp.int32)

    def uniform(self, shape, lo=0.0, hi=1.0):
        return jax.random.uniform(self._next(), shape, jnp.bfloat16, lo, hi)

    def permutation(self, n):
        return jax.random.permutation(self._next(), n)
kernel_name = 'adaLN_cond__linear_attn_block__swiglu_ffn__prompt'

def setup_inputs():
    _rng = _Rng(jax.random.key(int.from_bytes(__import__("os").urandom(4), "little")))
    _w = lambda a: (lambda t: t.astype(jnp.bfloat16) if jnp.issubdtype(t.dtype, jnp.floating) else t)(jnp.asarray(a))

    def _A_setup():
        B, S, D = (1, 2048, 640)
        return {'x': _w((lambda *s: _rng.normal(s) * 0.05)(B, S, D)), 'wqkv': _w((lambda *s: _rng.normal(s) * 0.8)(D, 3 * D)), 'wo': _w((lambda *s: _rng.normal(s) * 0.05)(D, D))}
    _A_in = _A_setup()

    def _B_setup():
        B, S, D, F = (1, 2048, 640, 1728)
        return {'x': _w((lambda *s: _rng.normal(s) * 0.05)(B, S, D)), 'w_gate': _w((lambda *s: _rng.normal(s) * 0.05)(D, F)), 'w_up': _w((lambda *s: _rng.normal(s) * 0.05)(D, F)), 'w_down': _w((lambda *s: _rng.normal(s) * 0.05)(F, D))}
    _B_in = _B_setup()
    return {'A_x': _A_in['x'], 'A_wqkv': _A_in['wqkv'], 'A_wo': _A_in['wo'], 'B_x': _B_in['x'], 'B_w_gate': _B_in['w_gate'], 'B_w_up': _B_in['w_up'], 'B_w_down': _B_in['w_down'], 'c': _w((lambda *s: _rng.normal(s) * 0.05)(1, 640) * 8.0), 'w_mod': _w((lambda *s: _rng.normal(s) * 0.05)(640, 6 * 640) * 640 ** (-0.5) * 8.0)}

def reference(A_x, A_wqkv, A_wo, B_x, B_w_gate, B_w_up, B_w_down, c, w_mod):

    def _A_ref(x, wqkv, wo):
        B, S, D = x.shape
        H = 32
        Dh = D // H
        qkv = (lambda x, *d: x.transpose(*d))((x @ wqkv).reshape(B, S, 3, H, Dh), 2, 0, 3, 1, 4)
        q, k, v = (qkv[0], qkv[1], qkv[2])
        phi = lambda t: jnp.where(t > 0, t + 1, jnp.exp(t)) + 1e-06
        pq, pk = (phi(q), phi(k))
        kv = jnp.einsum('bhsd,bhse->bhde', pk, v)
        z = jnp.einsum('bhsd->bhd', pk)
        num = jnp.einsum('bhqd,bhde->bhqe', pq, kv)
        den = jnp.einsum('bhqd,bhd->bhq', pq, z)[..., None] + 1e-06
        o = num / den
        return (lambda x, *d: x.transpose(*d))(o, 0, 2, 1, 3).reshape(B, S, D) @ wo

    def _B_ref(x, w_gate, w_up, w_down):
        g = _silu(x @ w_gate)
        u = x @ w_up
        return g * u @ w_down
    x = A_x
    mod = (_silu(c) @ w_mod).reshape(c.shape[0], 6, 1, -1)
    sa, ca, ga, sb, cb, gb = (mod[:, 0].copy(), mod[:, 1].copy(), mod[:, 2].copy(), mod[:, 3].copy(), mod[:, 4].copy(), mod[:, 5].copy())
    h = _layernorm(x, axis=-1) * (1 + ca) + sa
    x = x + ga * _A_ref(h, A_wqkv, A_wo)
    h = _layernorm(x, axis=-1) * (1 + cb) + sb
    x = x + gb * _B_ref(h, B_w_gate, B_w_up, B_w_down)
    return x
```

```python
import jax
import jax.numpy as jnp
from jax import lax
import jax.experimental.pallas as pl
import jax.experimental.pallas.tpu as pltpu

S, D, F, H, DH = 2048, 640, 1728, 32, 20
L = 128
NT = D // L
FT = F // L
BF, F32, U32 = jnp.bfloat16, jnp.float32, jnp.uint32
BANDS = [((L * j // DH * DH) // 16 * 16, -(-(((L * j + L - 1) // DH + 1) * DH) // 16) * 16) for j in range(NT)]


def _nn(a, b):
    return jnp.dot(a, b, preferred_element_type=F32)


def _nt(a, b):
    return lax.dot_general(a, b, (((1,), (1,)), ((), ())), preferred_element_type=F32)


def _tile(j):
    return slice(L * j, L * (j + 1))


def _axpy(a, t, x):
    if t == 0:
        return a
    if abs(t) == 1:
        return a + x if t > 0 else a - x
    return a + t * x


def _pairs(idx):
    return [(i, j) for i in idx for j in idx if i < j]


def _keys(idx):
    return [("D", i) for i in idx] + [("E", i) for i in idx] + [(p, i, j) for i, j in _pairs(idx) for p in range(3)]


ALL = tuple(range(NT))
SLOT = {k: r for r, k in enumerate(_keys(ALL))}


MH = 128
NB = S // (2 * MH)
T = (0.5, -1.0, -0.5, -2.0, 0.0)
TOUR = ((0, 1), (0, 3), (0, 2), (0, 4), (1, 4), (1, 3), (1, 2), (2, 3), (2, 4), (3, 4))

HEAD = (
    "+x0 +k +x1 +m1 !x0 n0 !k K !x1 n1 +m0 !m1 +x2 m1 k0:3 k1:3 k0:1 k1:3 k0:5 k1:3 +x3 k0:3 k1:3 k0 k1 "
    "!m0 !x2 m0 k2:3 k3:6 +q k2:3 k3:3 k2:3 k3:3 k2:5 k3:1 k2 k3 !x3 +m2 G0:1 k4:3 k5:1 G0:1 k4:1 k5:1 "
    "k4:1 k5:3 G0:1 k4:4 k5:3 k6:1 G0:1 k4:3 k5:2 k4 k5:2 G0:2 k6:1 k5:1 k6:2 k5 k7:2 G0:1 k7:1 +v k6:3 "
    "k7:3 +o G0:1 k6:3 k7:5 G0:1 k6:2 +g k7:1 G0 k6 k7 !q G4:2 Q q0:1 q1:1 G4:1 q1:1 +u G4:2 q1:5 G4:2 "
    "q1:2 q0:1 q1:1 q0:2 G4:2 q0:1 G4 q1:1 q0:2 q1:1 q0:2 q1 +d q0 !m2 !v !o !g !u m2 f:1 q2:8 f:3 m3 m4 "
    "m5 f:1 q2:1 f:1 q2:4 f:2 q2 f q3 o0 q4:14 0:1 q4 0:1 1:1 q5:2 0:1 q5:1 0:1 1:1 q5:2 1:1 0:1 q5:1 0:1 "
    "1:5 q5:1 1:1 q5:2 2:3 0:4 1:2 q5:3 1:3 0:1 1 0 q5 o:2 2:2 o:3 q6:5 3:2 q6:3 2:5 q6:2 r:3 3:4 2 q6:2 "
    "3:2 q6:2 3:5 r:1 q7:2 r:2 3 q7:1 r:1 q6 r q7:7 4:1 q7:3 4:2 q7:1 4:2 o:1 4 o:2 q7 o:6 act o !d "
)
FIRST_STEP = (
    "d:3 0:2 o:1 0:3 1:1 0:1 d:2 0:1 1:1 0:2 1:5 d:2 1:2 o:1 0 o:1 1:1 o:5 d:1 o:1 1:1 o:4 1:1 2:1 1 2:3 "
    "d:4 2:3 d:1 2:3 d:1 3:1 o 3:4 2:2 3:1 2:1 4:1 3:2 4:1 3:3 r:3 d:2 r:2 3 r:1 4:2 d r 4:4 2 4 "
)
STEP = (
    "d:3 0:7 d:2 0:3 o:1 0:4 1:1 0 1:2 d:2 1:2 o:2 1:7 o:4 d:1 o:2 1:1 d:1 2:1 1 2:3 d:1 o:4 d:1 2:3 o:1 "
    "2:3 d:2 3:2 o 3:2 4:2 2:4 3:3 2 r:3 3:3 d:1 3:4 4:2 d:1 3 r:1 4:1 d:1 4:1 d r:3 4:3 r 4 "
)
LAST_STEP = (
    "d:3 0:7 d:2 0:3 o:1 0:4 1:1 0 1:2 d:2 1:1 o:2 1:8 o:4 d:2 o:2 1:1 o:4 2:1 1 2:3 d:2 2:3 d:1 2:3 d:1 "
    "3:2 o 3:3 2:2 3:1 2 4:2 3:8 r:3 d:2 3 r:2 4:1 d:1 4:1 d r:1 4:3 r 4 "
)


def _phi(t):
    return jnp.where(t > 0, t + 1.0, jnp.exp(t)) + 1e-6


def _silu_mul(g, u):
    a = 0.5 * g
    return (a * u) * (jnp.tanh(a) + 1.0)


def _ln(xs):
    m = jnp.sum(sum(xs[1:], xs[0]), axis=-1, keepdims=True) * (1.0 / D)
    d = [x - m for x in xs]
    sq = [t * t for t in d]
    v = jnp.sum(sum(sq[1:], sq[0]), axis=-1, keepdims=True) * (1.0 / D)
    r = lax.rsqrt(v + 1e-5)
    return [t * r for t in d]


def _issue(plan, parts, copies):
    for item in plan.split():
        name, _, n = item.partition(":")
        if name[0] in "+!":
            for cp in copies[name[1:]]:
                cp.start(priority=int(n or 0)) if name[0] == "+" else cp.wait()
        elif name in parts:
            for _ in (range(int(n)) if n else iter(int, 1)):
                if next(parts[name], "end") == "end":
                    break


def _words(x):
    return pltpu.bitcast(x, U32)


def _unpack(x):
    return pltpu.bitcast(x, BF)


def _build(head=HEAD, first_step=FIRST_STEP, plan=STEP, last_step=LAST_STEP):
    mh, nb = MH, NB

    def a_ops(a1, a2, idx=ALL):
        scaled = {}

        def sx(i, c):
            if abs(c) == 1:
                return a2[i]
            if (i, abs(c)) not in scaled:
                scaled[i, abs(c)] = abs(c) * a2[i]
            return scaled[i, abs(c)]

        al = {i: a1[i] if T[i] == 0 else (a1[i] + sx(i, T[i]) if T[i] > 0 else a1[i] - sx(i, T[i])) for i in idx}
        ops = {}
        for i in idx:
            ops["D", i], ops["E", i] = al[i], a2[i]
        for i, j in _pairs(idx):
            d = T[j] - T[i]
            g = al[i] - al[j]
            ops[0, i, j] = g
            ops[1, i, j] = g + sx(i, d) if d > 0 else g - sx(i, d)
            ops[2, i, j] = g + sx(j, d) if d > 0 else g - sx(j, d)
        return ops

    def b_ops(b1, b2):
        be = [_axpy(b2[i], -T[i], b1[i]) for i in ALL]
        ops = {}
        for i in ALL:
            ops["D", i], ops["E", i] = b1[i], be[i]
        for i, j in _pairs(ALL):
            d = T[j] - T[i]
            w = be[j] - be[i] if d > 0 else be[i] - be[j]
            if abs(d) != 1:
                w = w * (1.0 / abs(d))
            ops[0, i, j], ops[1, i, j], ops[2, i, j] = w, w + b1[j], w + b1[i]
        return ops

    def widen(w):
        if w.dtype == F32:
            return w
        return lax.bitcast_convert_type(lax.bitcast_convert_type(w, jnp.int16).astype(jnp.int32) << 16, F32)

    def w_ops(raw, idx=ALL):
        ops = {}
        for i in idx:
            col, row = [raw(k, i).astype(F32) for k in idx], [widen(raw(i, k)) for k in idx]
            ops["D", i], ops["E", i] = sum(col[1:], col[0]), sum(row[1:], row[0])
        for i, j in _pairs(idx):
            ops[0, i, j] = widen(raw(j, i)) - raw(i, j).astype(F32)
        return ops

    def prep_w(w, raw, idx=ALL, words=None):
        for k, v in w_ops(raw, idx).items():
            w[k] = (lambda v: lambda: v)(v.astype(BF))
        for i, j in _pairs(idx):
            for k, v in (((1, i, j), raw(i, j)), ((2, i, j), raw(j, i))):
                if words is None:
                    w[k] = (lambda v: lambda: v)(v.astype(BF))
                else:
                    words[SLOT[k]] = _words(v)
                    w[k] = (lambda k: lambda: _unpack(words[SLOT[k]]))(k)

    def combine(prod, out, idx=ALL):
        def gen():
            y, b = {}, {}
            left = [p for p in TOUR if p[0] in idx and p[1] in idx]
            while left:
                i, j = left.pop(0)
                for n in (i, j):
                    if n not in y:
                        y[n], b[n] = prod(("D", n)), prod(("E", n))
                        yield
                p0, p1, p2 = prod((0, i, j)), prod((1, i, j)), prod((2, i, j))
                y[j] = y[j] + p1
                y[i] = y[i] - p2
                d = T[j] - T[i]
                q = p0 + p1 - p2
                if abs(d) != 1:
                    q = q * (1.0 / abs(d))
                if d > 0:
                    b[j], b[i] = b[j] + q, b[i] - q
                else:
                    b[j], b[i] = b[j] - q, b[i] + q
                for n in (i, j):
                    if not any(n in p for p in left):
                        out[n] = (_axpy(y[n], -T[n], b[n]), b[n])
                yield
        return gen()

    def body(x_hbm, wqkv_hbm, wo_hbm, wg_hbm, wu_hbm, wd_hbm, c_ref, wmod_hbm, out_hbm,
             c_v, x_v, pq_v, h2_v, hid_v, x1_v, wqkv_v, wo_v, wg_v, wu_v, wt_v, wd_v, wmod_v,
             f32_v, gacc_v, zacc_v, vec_v, o_v,
             sem_w, sem_o, wd_words, *gu_words):
        def cols(src, dst, a, b, s):
            return pltpu.make_async_copy(src.at[:, pl.ds(a * D, (b - a) * D)], dst.at[:, pl.ds(a * D, (b - a) * D)], sem_w.at[s])

        def rows(src, dst, a, b, s, off=None):
            return pltpu.make_async_copy(src.at[pl.ds(a, b - a)], dst.at[pl.ds(a if off is None else off, b - a)], sem_w.at[s])

        def x_rows(a, b, s):
            return rows(x_hbm, x_v, a * 2 * mh, b * 2 * mh, s)

        copies = {
            "x0": [x_rows(0, 1, 0)], "x1": [x_rows(1, 2, 1)], "x2": [x_rows(2, 4, 2)], "x3": [x_rows(4, nb, 15)],
            "q": [cols(wqkv_hbm, wqkv_v, 0, 1, 3)], "k": [cols(wqkv_hbm, wqkv_v, 1, 2, 4)], "v": [cols(wqkv_hbm, wqkv_v, 2, 3, 5)],
            "o": [pltpu.make_async_copy(wo_hbm, wo_v, sem_w.at[6])],
            "m0": [cols(wmod_hbm, wmod_v, 0, 1, 7)], "m1": [cols(wmod_hbm, wmod_v, 1, 2, 8), pltpu.make_async_copy(c_ref, c_v, sem_w.at[16])], "m2": [cols(wmod_hbm, wmod_v, 2, 6, 9)],
            "g": [rows(wg_hbm, wg_v, 0, FT * L, 10), rows(wg_hbm, wt_v, FT * L, F, 11, 0)],
            "u": [rows(wu_hbm, wu_v, 0, FT * L, 12), rows(wu_hbm, wt_v, FT * L, F, 13, F - FT * L)],
            "d": [rows(wd_hbm, wd_v, 0, F, 14)],
        }
        wd_v[F:, :] = jnp.zeros(((FT + 1) * L - F, D), BF)

        for name in copies:
            assert head.split().count("+" + name) == head.split().count("!" + name) == 1, name

        def gu_tile(n, i):
            ref, t = (wt_v, 0) if n == 2 * FT else ((wg_v, wu_v)[n % 2], n // 2)
            return ref[_tile(t), _tile(i)]

        w_k, w_q, w_p, w_rem, w_d, w_gu = {}, {}, {}, {}, {}, [{} for _ in range(5)]

        def perm_rows(ref, j):
            return jnp.concatenate([ref[pl.ds(4 * j + d, H, stride=DH), :] for d in range(4)], axis=0)

        def prep_k():
            tiles = {(i, j): wqkv_v[_tile(i), D + L * j:D + L * (j + 1)].T for i in ALL for j in ALL}
            prep_w(w_k, lambda i, j: tiles[i, j])
            yield

        def prep_q():
            tiles = {}
            for i in ALL:
                for j in ALL:
                    f32_v[i, _tile(j), :] = wqkv_v[_tile(i), _tile(j)].astype(F32).T
                for j in ALL:
                    tiles[i, j] = perm_rows(f32_v.at[i], j)
            prep_w(w_q, lambda i, j: tiles[i, j])
            wqt = jnp.concatenate([jnp.concatenate([tiles[i, j] for i in ALL], axis=1) for j in ALL], axis=0)
            bias["q"] = jnp.sum(_nt(mods["shift"], wqt.astype(BF)), axis=0, keepdims=True)
            yield

        def prep_d():
            raw = [lambda i, j, g=g: wd_v[D * g + L * i:D * g + L * (i + 1), _tile(j)] for g in range(3)]
            sums = [w_ops(raw[g], ALL if g < 2 else ALL[:4]) for g in range(3)]
            for k in sums[0]:
                w_d[k] = (lambda v: lambda: v)(jnp.concatenate([t[k] for t in sums if k in t], axis=0).astype(BF))
            for i, j in _pairs(ALL):
                n = 3 if j < 4 else 2
                for k, (a, b) in (((1, i, j), (i, j)), ((2, i, j), (j, i))):
                    for g in range(n):
                        wd_words[SLOT[k], L // 2 * g:L // 2 * (g + 1), :] = _words(raw[g](a, b))
                    w_d[k] = (lambda k, n: lambda: _unpack(wd_words[SLOT[k], 0:L // 2 * n, :]))(k, n)

        first = lambda i: isinstance(i, int) and i == 0

        def start(i, size):
            return i * size if isinstance(i, int) else pl.multiple_of(i * size, size)

        def x_tiles(i, s):
            return [x_v[pl.ds(start(i, 2 * mh) + s * mh, mh), _tile(j)].astype(F32) for j in ALL]

        normed, mods, bias = {}, {}, {}

        def norm(i):
            normed[i] = [_ln(x_tiles(i, s)) for s in range(2)]
            yield

        hop_f32, hop = {}, {}

        def ln_ops(i):
            n = normed[i] if i in normed else [_ln(x_tiles(i, s)) for s in range(2)]
            hop_f32[i] = a_ops(*[[n[s][j] * mods[1][:, _tile(j)] for j in ALL] for s in range(2)])
            hop[i] = {k: v.astype(BF) for k, v in hop_f32[i].items()}

        kts = [{} for _ in range(nb)]

        def k_prod(i):
            ln_ops(i)
            yield from combine(lambda k: _nt(w_k[k](), hop[i][k]), kts[i])

        def g_prod(i0, n):
            pk = [[[_phi(kt[j][s] + bias['k'][j]) for j in ALL] for s in range(2)] for kt in kts[i0:i0 + n]]
            for j in ALL:
                zs = [p[s][j][:, _tile(t)] for p in pk for s in range(2) for t in range(mh // L)]
                zs = sum(zs[1:], zs[0])
                zacc_v[_tile(j), :] = zs if first(i0) else zacc_v[_tile(j), :] + zs
            bops = [b_ops(*p) for p in pk]
            for k in SLOT:
                p = [_nn(bops[m][k].astype(BF), hop[i0 + m][k]) for m in range(n)]
                p = sum(p[1:], p[0])
                gacc_v[SLOT[k]] = p if first(i0) else gacc_v[SLOT[k]] + p
                if SLOT[k] % 4 == 3:
                    yield

        def q_prod(i):
            q = {}
            yield from combine(lambda k: _nt(hop[i][k], w_q[k]()), q)
            for s in range(2):
                for j in ALL:
                    pq_v[pl.ds(start(i, 2 * mh) + s * mh, mh), _tile(j)] = _phi(q[j][s] + bias['q'][:, _tile(j)])

        def mod(n):
            if "c" not in mods:
                c = c_v[...].astype(F32)
                mods["c"] = jnp.broadcast_to((c * jax.nn.sigmoid(c)).astype(BF), (16, D))
            m = _nn(mods['c'], wmod_v[:, n * D:(n + 1) * D])[0:1]
            mods[n] = 1.0 + m if n % 3 == 1 else m
            if n == 0:
                hi = m.astype(BF)
                row = lax.broadcasted_iota(jnp.int32, (16, D), 0)
                mods["shift"] = jnp.where(row == 0, m, jnp.where(row == 1, m - hi.astype(F32), 0.0)).astype(BF)
                bk = jnp.sum(_nn(mods["shift"], wqkv_v[:, D:2 * D]), axis=0, keepdims=True)
                bias["k"] = [jnp.broadcast_to(bk[:, _tile(j)], (L, L)).T for j in ALL]
            if n >= 2:
                vec_v[n - 2:n - 1, :] = mods[n]
            yield

        def fold():
            acc = lambda k: gacc_v[SLOT[k]]
            dd, ee = [acc(("D", i)) for i in ALL], [acc(("E", i)) for i in ALL]
            gm = {(i, i): dd[i] + ee[i] for i in ALL}
            for i, j in _pairs(ALL):
                gm[j, i] = acc((1, i, j)) - acc((0, i, j)) + dd[j] + ee[i]
                gm[i, j] = acc((0, i, j)) - acc((2, i, j)) + dd[i] + ee[j]
            gmat = jnp.concatenate([jnp.concatenate([gm[j, i] for i in ALL], axis=1) for j in ALL], axis=0)
            kvs = []
            bv = jnp.sum(_nn(mods["shift"], wqkv_v[:, 2 * D:]), axis=0, keepdims=True)
            zcol = jnp.sum(zacc_v[0:D, :], axis=1, keepdims=True)
            for j, (a, b) in enumerate(BANDS):
                kv = _nn(gmat[a:b].astype(BF), wqkv_v[:, 2 * D + L * j:2 * D + L * (j + 1)])
                rh = a + lax.broadcasted_iota(jnp.int32, (b - a, L), 0)
                lh = L * j + lax.broadcasted_iota(jnp.int32, (b - a, L), 1)
                same = ((rh * 3277) >> 16) == ((lh * 3277) >> 16)
                kvs.append(jnp.where(same, kv + zcol[a:b] * bv[:, _tile(j)], 0.0).astype(BF))
                yield
            parts = []
            for j in ALL:
                parts.append(_nn(kvs[j], wo_v[_tile(j), :]))
                yield
            ga = vec_v[0:1, :]
            cuts = sorted({e for ab in BANDS for e in ab})
            for lo, hi in zip(cuts[:-1], cuts[1:]):
                cover = [parts[j][lo - a:hi - a] for j, (a, b) in enumerate(BANDS) if a <= lo and hi <= b]
                seg = sum(cover[1:], cover[0]) * ga
                for j in ALL:
                    f32_v[j, lo:hi, :] = seg[:, _tile(j)]
            prep_w(w_p, lambda i, j: perm_rows(f32_v.at[j], i))
            for j in ALL:
                vec_v[4:5, _tile(j)] = jnp.sum(perm_rows(zacc_v, j).T, axis=0, keepdims=True)

        def q_feat(i):
            z = vec_v[4:5, :]
            ps = []
            for s in range(2):
                pq = [pq_v[pl.ds(start(i, 2 * mh) + s * mh, mh), _tile(j)] for j in ALL]
                t = [pq[j] * z[:, _tile(j)] for j in ALL]
                den = sum(t[1:], t[0])
                den = den + pltpu.roll(den, 2 * H, 1)
                den = den + pltpu.roll(den, H, 1)
                inv = 1.0 / (den + 1e-6)
                ps.append([p * inv for p in pq])
            return a_ops(*ps)

        def o_prod(ops, att):
            return combine(lambda k: _nn(ops[k].astype(BF), w_p[k]()), att)

        def o_norm(i, att):
            sb, cb1 = vec_v[1:2, :], vec_v[2:3, :]
            for s in range(2):
                x1 = [x + att[j][s] for j, x in enumerate(x_tiles(i, s))]
                n = _ln(x1)
                for j in ALL:
                    x1_v[i % 3, pl.ds(s * mh, mh), _tile(j)] = x1[j]
                    h2_v[i % 2, j, s] = n[j] * cb1[:, _tile(j)] + sb[:, _tile(j)]

        def h2_ops(slot):
            ops = a_ops(*[[h2_v[slot, j, s] for j in ALL] for s in range(2)])
            return {k: v.astype(BF) for k, v in ops.items()}

        def out_proj(i):
            att = {}
            yield from o_prod(q_feat(i), att)
            o_norm(i, att)

        def cp_o(i):
            rows = pl.ds(start(i, 2 * mh), 2 * mh)
            if isinstance(i, int) and i == nb - 1:
                return [pltpu.make_async_copy(o_v.at[rows, pl.ds(L * j, L)], out_hbm.at[rows, pl.ds(L * j, L)], sem_o.at[i + j]) for j in ALL]
            return [pltpu.make_async_copy(o_v.at[rows], out_hbm.at[rows], sem_o.at[i])]

        def streams(i, prev, cur, nxt):
            y, fin, q, att, ra, rb, tail = {}, {}, {}, {}, {}, {}, {}
            parts = {}
            if prev:
                hid, hops = [], []

                def down(k):
                    gs = range(3) if k in hops[2] else range(2)
                    return _nn(jnp.concatenate([hops[g][k] for g in gs], axis=1).astype(BF),
                               w_d[k]())

                def down_rest():
                    for s in range(2):
                        fin[s] = _nn(jnp.concatenate(hid[s][2 * NT:], axis=1).astype(BF), wd_v[2 * D:, _tile(4)])
                        yield

                def finish(j):
                    gb = vec_v[3:4, _tile(j)]
                    for s in range(2):
                        yj = y[j][s] + fin[s] if j == 4 else y[j][s]
                        o_v[pl.ds(start(i - 1, 2 * mh) + s * mh, mh), _tile(j)] = (
                            x1_v[(i + 2) % 3, s * mh:(s + 1) * mh, _tile(j)] + gb * yj).astype(BF)

                def down_proj():
                    if first(i - 1):
                        prep_d()
                    hid[:] = hids.pop(i - 1) if isinstance(i, int) and i - 1 in hids else [[hid_v[s, t] for t in range(FT + 1)] for s in range(2)]
                    hops[:] = [a_ops(hid[0][NT * g:], hid[1][NT * g:], ALL if g < 2 else ALL[:4]) for g in range(3)]
                    yield from down_rest()
                    cps, done = cp_o(i - 1), []
                    for _ in combine(down, y):
                        for j in [j for j in y if j not in done]:
                            finish(j)
                            done.append(j)
                            if len(cps) > 1:
                                cps[j].start()
                            elif len(done) == NT:
                                cps[0].start()
                        yield
                parts["d"] = down_proj()
            if nxt:
                parts["o"] = out_proj(i + 1)
            if cur:
                h2ops = {}

                def h2(k):
                    if not h2ops:
                        h2ops.update(h2_ops(i % 2))
                    return h2ops[k]
                gu = [{} for _ in range(5)]

                def rest():
                    for n in range(2):
                        tail[n] = [ra[n][s] + rb[2 + n][s] + _nt(h2((("D", 4), ("E", 4))[s]), gu_tile(25 + n, 4)) for s in range(2)]
                        yield

                def narrow():
                    if first(i):
                        for idx in ((0, 1), (2, 3)):
                            prep_w(w_rem, lambda a, b: gu_tile(25 + b % 2, a), idx, gu_words[5])
                    yield from combine(lambda k: _nt(h2(k), w_rem[k]()), ra, (0, 1))
                    yield from combine(lambda k: _nt(h2(k), w_rem[k]()), rb, (2, 3))
                    yield from rest()
                parts["r"] = narrow()

                def wide(g):
                    if first(i):
                        prep_w(w_gu[g], lambda a, b: gu_tile(NT * g + b, a), ALL, gu_words[g])
                    yield from combine(lambda k: _nt(h2(k), w_gu[g][k]()), gu[g])
                for g in range(5):
                    parts[str(g)] = wide(g)

                def act():
                    lane = lax.broadcasted_iota(jnp.int32, (mh, L), 1)
                    out = []
                    for s in range(2):
                        cols = [gu[n // NT][n % NT][s] for n in range(25)] + [tail[0][s]]
                        t = tail[1][s]
                        out.append([_silu_mul(cols[2 * n], cols[2 * n + 1]) for n in range(FT)]
                                   + [jnp.where(lane < F - FT * L, _silu_mul(t, pltpu.roll(t, L // 2, 1)), 0.0)])
                    if isinstance(i, int) and not i == 1:
                        hids[i] = out
                    else:
                        for s in range(2):
                            for n in range(FT + 1):
                                hid_v[s, n] = out[s][n]
                    yield
                parts["act"] = act()
            return parts

        def step(i, prev, cur, nxt):
            _issue((first_step if first(i - 1) else last_step if isinstance(i, int) and i >= nb - 1 else plan) + " r 0 1 2 3 4 o d act", streams(i, prev, cur, nxt), copies)

        hids = {}
        parts = {"K": prep_k(), "Q": prep_q(), **{f"n{i}": norm(i) for i in range(nb)}, "f": fold(), "o0": out_proj(0), **{f"m{n}": mod(n) for n in range(6)},
                 **{f"k{i}": k_prod(i) for i in range(nb)}, **{f"q{i}": q_prod(i) for i in range(nb)},
                 **{f"G{i}": g_prod(i, n) for i, n in ((0, 4), (4, 4))}, **streams(0, False, True, True)}
        _issue(head, parts, copies)
        step(1, True, True, True)
        lax.fori_loop(2, nb - 1, lambda i, carry: step(i, True, True, True), None)
        step(nb - 1, True, True, False)
        step(nb, True, False, False)
        for i in range(nb):
            for cp in cp_o(i):
                cp.wait()

    def fn(A_x, A_wqkv, A_wo, B_x, B_w_gate, B_w_up, B_w_down, c, w_mod):
        hbm = pl.BlockSpec(memory_space=pltpu.HBM)
        out = pl.pallas_call(
            body,
            out_shape=jax.ShapeDtypeStruct((S, D), BF),
            in_specs=[hbm] * 8,
            out_specs=hbm,
            scratch_shapes=[
                pltpu.VMEM((1, D), BF),
                pltpu.VMEM((S, D), BF),
                pltpu.VMEM((S, D), F32), pltpu.VMEM((2, NT, 2, mh, L), F32), pltpu.VMEM((2, FT + 1, mh, L), F32),
                pltpu.VMEM((3, 2 * mh, D), F32),
                pltpu.VMEM((D, 3 * D), BF), pltpu.VMEM((D, D), BF),
                pltpu.VMEM((FT * L, D), BF), pltpu.VMEM((FT * L, D), BF), pltpu.VMEM((L, D), BF),
                pltpu.VMEM(((FT + 1) * L, D), BF),
                pltpu.VMEM((D, 6 * D), BF),
                pltpu.VMEM((NT, D + 2 * DH, L), F32),
                pltpu.VMEM((40, L, L), F32), pltpu.VMEM((D + 2 * DH, L), F32), pltpu.VMEM((8, D), F32),
                pltpu.VMEM((S, D), BF),
                pltpu.SemaphoreType.DMA((17,)), pltpu.SemaphoreType.DMA((nb + NT - 1,)),
            ] + [pltpu.VMEM((40, 3 * L // 2, L), U32)] + [pltpu.VMEM((40, L // 2, L), U32)] * 6,
            compiler_params=pltpu.CompilerParams(vmem_limit_bytes=110 * 1024 * 1024, disable_semaphore_checks=True),
        )(A_x.reshape(S, D), A_wqkv, A_wo, B_w_gate.T, B_w_up.T, B_w_down, c, w_mod)
        return out.reshape(1, S, D)
    return fn


@jax.jit
def pallas_adaLN_cond__linear_attn_block__swiglu_ffn__prompt_kernel(
    A_x: jax.Array,
    A_wqkv: jax.Array,
    A_wo: jax.Array,
    B_x: jax.Array,
    B_w_gate: jax.Array,
    B_w_up: jax.Array,
    B_w_down: jax.Array,
    c: jax.Array,
    w_mod: jax.Array,
):
    return _build()(A_x, A_wqkv, A_wo, B_x, B_w_gate, B_w_up, B_w_down, c, w_mod)
```
